```python
import jax
import jax.numpy as jnp

def _softmax(x, axis=-1):
    return jax.nn.softmax(x, axis=axis)

def _gelu(x):
    return jax.nn.gelu(x, approximate=True)

def _silu(x):
    return jax.nn.silu(x)

def _sigmoid(x):
    return jax.nn.sigmoid(x)

def _layernorm(x, axis=-1, eps=1e-05):
    m = jnp.mean(x, axis=axis, keepdims=True)
    v = jnp.var(x, axis=axis, keepdims=True)
    return (x - m) / jnp.sqrt(v + eps)

def _scatter_add(tgt, idx, src, axis=0):
    return tgt.at[idx].add(src)

def _segment_sum(src, seg, n):
    return jax.ops.segment_sum(src, seg, n)

class _Rng:

    def __init__(self, key):
        self._k = key

    def _next(self):
        self._k, sub = jax.random.split(self._k)
        return sub

    def normal(self, shape):
        return jax.random.normal(self._next(), shape, dtype=jnp.bfloat16)

    def randint(self, lo, hi, shape):
        return jax.random.randint(self._next(), shape, lo, hi, dtype=jnp.int32)

    def uniform(self, shape, lo=0.0, hi=1.0):
        return jax.random.uniform(self._next(), shape, jnp.bfloat16, lo, hi)

    def permutation(self, n):
        return jax.random.permutation(self._next(), n)
kernel_name = 'standalone__dilated_atrous__vision'

def setup_inputs():
    _rng = _Rng(jax.random.key(int.from_bytes(__import__("os").urandom(4), "little")))
    _w = lambda a: (lambda t: t.astype(jnp.bfloat16) if jnp.issubdtype(t.dtype, jnp.floating) else t)(jnp.asarray(a))
    H = W = 384
    C = 384
    k = 1
    return {'x': _w((lambda *s: _rng.normal(s) * 0.05)(1, H, W, C)), 'w': _w((lambda *s: _rng.normal(s) * 0.05)(k, k, C, C) * (1.0 / (k * C ** 0.5)))}

def reference(x, w):
    B, H, W, C = x.shape
    k = 1
    rate = 2
    pad = (k - 1) * rate // 2
    xp = jnp.pad(x, ((0, 0), (pad, pad), (pad, pad), (0, 0)))
    out = jnp.zeros_like(x)
    for i in range(k):
        for j in range(k):
            tap = xp[:, i * rate:i * rate + H, j * rate:j * rate + W, :].copy()
            out = out + jnp.einsum('bhwc,co->bhwo', tap, w[i, j])
    return out
```

```python
import jax
import jax.numpy as jnp
from jax import lax
import jax.experimental.pallas as pl
import jax.experimental.pallas.tpu as pltpu

_SLAB = 4096
_PIECE = 64
_R_SLABS = 12
_W_SLABS = 6
_SMALL = 32
_TM = 1024
_CHUNK = 128

_SPLIT = 3
_LEAD = 9
_PRE = 74
_BOOST = 10
_BIG_16 = 101
_SMALL_PER_STEP = 19
_TAIL = 2
_W_FIRST = 12
_W_PER_STEP = 14


def _split(i, n):
    assert n & (n - 1) == 0
    return lax.shift_right_logical(i, n.bit_length() - 1), i & (n - 1)


@jax.jit
def pallas_standalone__dilated_atrous__vision_kernel(
    x: jax.Array,
    w: jax.Array,
):
    B, H, W, C = x.shape
    assert w.shape == (1, 1, C, C) and C % 128 == 0
    M = B * H * W
    blocks = C // 128
    n_slabs = M * blocks // _SLAB
    n_steps = M // _TM
    pieces = _SLAB // _PIECE
    assert n_slabs * _SLAB == M * blocks and n_steps * _TM == M

    n_groups = n_slabs // _R_SLABS
    n_big = (n_groups - 1) * pieces
    n_small = _R_SLABS * _SLAB // _SMALL
    group_steps = _R_SLABS * _SLAB // (blocks * _TM)
    big_pre = _PRE + _BOOST
    small_pre = (_PRE - _LEAD) * _SPLIT + _BOOST
    n1 = (n_small - small_pre) // _SMALL_PER_STEP
    assert n_groups * _R_SLABS == n_slabs and group_steps * n_groups == n_steps
    assert big_pre + n1 * _BIG_16 // 16 >= n_big
    assert pl.cdiv(n1, group_steps) <= n_groups - 2
    assert big_pre >= pieces and group_steps * _BIG_16 // 16 >= pieces

    n_writes = n_slabs // _W_SLABS * pieces
    write_steps = _W_SLABS * _SLAB // (blocks * _TM)
    assert write_steps * n_slabs == n_steps * _W_SLABS
    assert _W_FIRST <= n1 // write_steps * pieces

    def kernel_function(x_hbm, w_hbm, o_hbm, buf, wbuf, in_sems, sems):
        def read(idx, sem):
            return pltpu.make_async_copy(x_hbm.at[idx], buf.at[idx], in_sems.at[sem])

        def piece(j):
            return pl.ds(pl.multiple_of(j * _PIECE, _PIECE), _PIECE)

        def start_big(k):
            g, j = _split(k, pieces)
            sem = jnp.where(k >= n_big - _TAIL, n_groups, g)
            read((pl.ds(g * _R_SLABS, _R_SLABS), piece(j)), sem).start(priority=1)

        def start_part(k, part):
            g, j = _split(k, pieces)
            n = _R_SLABS // _SPLIT
            read((pl.ds(g * _R_SLABS + part * n, n), piece(j)), g).start(priority=1)

        def start_small(m):
            s, r = _split(m, _SLAB // _SMALL)
            lines = pl.ds(pl.multiple_of(r * _SMALL, _SMALL), _SMALL)
            read((n_slabs - _R_SLABS + s, lines), n_groups - 1).start()

        def wait_reads(g, sem, lo=0, hi=_SLAB):
            read((pl.ds(g * _R_SLABS, _R_SLABS), pl.ds(lo, hi - lo)), sem).wait()

        def start_writes(lo, hi):
            def start(k, _):
                g, j = _split(k, pieces)
                idx = (pl.ds(g * _W_SLABS, _W_SLABS), piece(j))
                pltpu.make_async_copy(buf.at[idx], o_hbm.at[idx], sems.at[1]).start()

            lax.fori_loop(lo, hi, start, None)

        rows16 = buf.reshape(M // 16, 16 * blocks, 128)

        def tiles(i, k, c):
            units = pl.ds(i * (_TM // 16) + k * (_CHUNK // 16), _CHUNK // 16)
            return [(units, pl.ds(8 * (half * blocks + c), 8)) for half in range(2)]

        def matmul_step(i, before_store):
            def product(k):
                cols = [jnp.concatenate([rows16[t] for t in tiles(i, k, c)], axis=1)
                        for c in range(blocks)]
                lhs = jnp.concatenate([v.reshape(_CHUNK, 128) for v in cols], axis=1)
                res = jnp.dot(lhs, wbuf[...], preferred_element_type=jnp.float32)
                return res.astype(buf.dtype)

            def store(k, res):
                for c in range(blocks):
                    before_store(k * blocks + c)
                    v = res[:, c * 128:(c + 1) * 128].reshape(_CHUNK // 16, 16, 128)
                    for half, t in enumerate(tiles(i, k, c)):
                        rows16[t] = v[:, 8 * half:8 * half + 8]

            res = product(0)
            for k in range(1, _TM // _CHUNK):
                res, done = product(k), res
                store(k - 1, done)
            store(_TM // _CHUNK - 1, res)

        w_copy = pltpu.make_async_copy(w_hbm, wbuf, sems.at[0])
        w_copy.start(priority=1)

        def lead(k, _):
            for part in range(_SPLIT):
                start_part(k, part)

        def pre(k, _):
            for part in range(_SPLIT):
                start_part(k, part)
                start_small((k - _LEAD) * _SPLIT + part)

        def boost(k, _):
            start_big(_PRE + k)
            start_small(small_pre - _BOOST + k)

        lax.fori_loop(0, _LEAD, lead, None)
        lax.fori_loop(_LEAD, _PRE, pre, None)
        lax.fori_loop(0, _BOOST, boost, None)
        w_copy.wait()

        def read_step(i, _):
            g, r = _split(i, group_steps)
            pl.when(r == 0)(lambda: wait_reads(g, g))
            lo = big_pre + _split(i * _BIG_16, 16)[0]
            hi = big_pre + _split((i + 1) * _BIG_16, 16)[0]
            lax.fori_loop(lo, jnp.minimum(hi, n_big), lambda k, _: start_big(k), None)

            stores = _TM // _CHUNK * blocks

            def before_store(p):
                for q in range(_SMALL_PER_STEP):
                    if (q * stores + 6) // _SMALL_PER_STEP == p:
                        start_small(small_pre + i * _SMALL_PER_STEP + q)

            matmul_step(i, before_store)

        lax.fori_loop(0, n1, read_step, None)
        lax.fori_loop(small_pre + n1 * _SMALL_PER_STEP, n_small,
                      lambda m, _: start_small(m), None)

        for g in range(pl.cdiv(n1, group_steps), n_groups - 2):
            wait_reads(g, g)
        tail = _SLAB - _TAIL * _PIECE
        wait_reads(n_groups - 2, n_groups - 2, hi=tail)
        start_writes(0, _W_FIRST)
        wait_reads(n_groups - 2, n_groups, lo=tail)
        wait_reads(n_groups - 1, n_groups - 1)

        def write_step(i, started):
            ready = _split(i, write_steps)[0] * pieces
            target = jnp.minimum(ready, _W_FIRST + (i - n1 + 1) * _W_PER_STEP)
            start_writes(started, target)
            matmul_step(i, lambda p: None)
            return target

        started = lax.fori_loop(n1, n_steps, write_step, jnp.int32(_W_FIRST))
        start_writes(started, n_writes)
        pltpu.make_async_copy(buf, o_hbm, sems.at[1]).wait()

    lines = x.reshape(M // 8, 8, blocks, 128).swapaxes(1, 2)
    out = pl.pallas_call(
        kernel_function,
        in_specs=[
            pl.BlockSpec(memory_space=pl.ANY),
            pl.BlockSpec(memory_space=pl.ANY),
        ],
        out_specs=pl.BlockSpec(memory_space=pl.ANY),
        out_shape=jax.ShapeDtypeStruct((n_slabs, _SLAB, 128), x.dtype),
        scratch_shapes=[
            pltpu.VMEM((n_slabs, _SLAB, 128), x.dtype),
            pltpu.VMEM((C, C), w.dtype),
            pltpu.SemaphoreType.DMA((n_groups + 1,)),
            pltpu.SemaphoreType.DMA((2,)),
        ],
        compiler_params=pltpu.CompilerParams(
            vmem_limit_bytes=120 * 2**20,
            disable_bounds_checks=True,
            disable_semaphore_checks=True,
        ),
    )(lines.reshape(n_slabs, _SLAB, 128), w.reshape(C, C))
    return out.reshape(M // 8, blocks, 8, 128).swapaxes(1, 2).reshape(B, H, W, C)
```

```python
import jax
import jax.numpy as jnp
from jax import lax
import jax.experimental.pallas as pl
import jax.experimental.pallas.tpu as pltpu

_SLAB = 4096
_PIECE = 64
_R_SLABS = 12
_W_SLABS = 6
_SMALL = 32
_TM = 1024
_CHUNK = 128

_SPLIT = 3
_LEAD = 9
_PRE = 78
_BOOST = 9
_BIG_16 = 102
_TAIL = 2
_W_FIRST = 24
_W_PER_STEP = 14


def _split(i, n):
    assert n & (n - 1) == 0
    return lax.shift_right_logical(i, n.bit_length() - 1), i & (n - 1)


@jax.jit
def pallas_standalone__dilated_atrous__vision_kernel(
    x: jax.Array,
    w: jax.Array,
):
    B, H, W, C = x.shape
    assert w.shape == (1, 1, C, C) and C % 128 == 0
    M = B * H * W
    blocks = C // 128
    n_slabs = M * blocks // _SLAB
    n_steps = M // _TM
    chunks = _TM // _CHUNK
    pieces = _SLAB // _PIECE
    assert n_slabs * _SLAB == M * blocks and n_steps * _TM == M

    n_groups = n_slabs // _R_SLABS
    n_big = (n_groups - 1) * pieces
    n_small = _R_SLABS * _SLAB // _SMALL
    group_steps = _R_SLABS * _SLAB // (blocks * _TM)
    big_pre = _PRE + _BOOST
    small_pre = _LEAD + (_PRE - _LEAD) * _SPLIT + _BOOST
    step_smalls = chunks * (blocks - 1) + 3
    n1 = (n_small - small_pre) // step_smalls
    assert n_groups * _R_SLABS == n_slabs and group_steps * n_groups == n_steps
    assert small_pre + n1 * step_smalls == n_small
    assert big_pre + (n1 - 1) * _BIG_16 // 16 >= n_big
    assert pl.cdiv(n1, group_steps) <= n_groups - 2
    assert big_pre >= pieces and group_steps * _BIG_16 // 16 >= pieces

    n_writes = n_slabs // _W_SLABS * pieces
    write_steps = _W_SLABS * _SLAB // (blocks * _TM)
    assert write_steps * n_slabs == n_steps * _W_SLABS
    assert _W_FIRST <= n1 // write_steps * pieces

    def kernel_function(x_hbm, w_hbm, o_hbm, buf, wbuf, in_sems, sems):
        def read(idx, sem):
            return pltpu.make_async_copy(x_hbm.at[idx], buf.at[idx], in_sems.at[sem])

        def piece(j):
            return pl.ds(pl.multiple_of(j * _PIECE, _PIECE), _PIECE)

        def start_big(k):
            g, j = _split(k, pieces)
            sem = jnp.where(k >= n_big - _TAIL, n_groups, g)
            read((pl.ds(g * _R_SLABS, _R_SLABS), piece(j)), sem).start(priority=1)

        def start_part(k, part):
            g, j = _split(k, pieces)
            n = _R_SLABS // _SPLIT
            read((pl.ds(g * _R_SLABS + part * n, n), piece(j)), g).start(priority=1)

        def start_small(m):
            m, r = _split(m, _PIECE // _SMALL)
            m, s = _split(m, 2)
            pair, j = _split(m, pieces)
            lines = pl.ds(pl.multiple_of(j * _PIECE + r * _SMALL, _SMALL), _SMALL)
            read((n_slabs - _R_SLABS + 2 * pair + s, lines), n_groups - 1).start()

        def wait_reads(g, sem, lo=0, hi=_SLAB):
            read((pl.ds(g * _R_SLABS, _R_SLABS), pl.ds(lo, hi - lo)), sem).wait()

        def start_writes(lo, hi):
            def start(k, _):
                g, j = _split(k, pieces)
                idx = (pl.ds(g * _W_SLABS, _W_SLABS), piece(j))
                pltpu.make_async_copy(buf.at[idx], o_hbm.at[idx], sems.at[1]).start()

            lax.fori_loop(lo, hi, start, None)

        rows16 = buf.reshape(M // 16, 16 * blocks, 128)

        def tiles(i, k, c):
            units = pl.ds(i * (_TM // 16) + k * (_CHUNK // 16), _CHUNK // 16)
            return [(units, pl.ds(8 * (half * blocks + c), 8)) for half in range(2)]

        def matmul_step(i, tick):
            def product(k):
                cols = [jnp.concatenate([rows16[t] for t in tiles(i, k, c)], axis=1)
                        for c in range(blocks)]
                lhs = jnp.concatenate([v.reshape(_CHUNK, 128) for v in cols], axis=1)
                res = jnp.dot(lhs, wbuf[...], preferred_element_type=jnp.float32)
                return res.astype(buf.dtype)

            def store(k, res):
                for c in range(blocks):
                    if c < blocks - 1:
                        tick()
                    v = res[:, c * 128:(c + 1) * 128].reshape(_CHUNK // 16, 16, 128)
                    for half, t in enumerate(tiles(i, k, c)):
                        rows16[t] = v[:, 8 * half:8 * half + 8]

            res = product(0)
            tick()
            for k in range(1, chunks):
                res, done = product(k), res
                store(k - 1, done)
            store(chunks - 1, res)
            tick()

        w_copy = pltpu.make_async_copy(w_hbm, wbuf, sems.at[0])
        w_copy.start(priority=1)

        def lead(k, _):
            for part in range(_SPLIT):
                start_part(k, part)
            start_small(k)

        def pre(k, _):
            for part in range(_SPLIT):
                start_part(k, part)
                start_small(_LEAD + (k - _LEAD) * _SPLIT + part)

        def boost(k, _):
            start_big(_PRE + k)
            start_small(small_pre - _BOOST + k)

        lax.fori_loop(0, _LEAD, lead, None)
        lax.fori_loop(_LEAD, _PRE, pre, None)
        lax.fori_loop(0, _BOOST, boost, None)
        w_copy.wait()

        def read_step(i, _):
            lo = big_pre + _split(jnp.maximum(i - 1, 0) * _BIG_16, 16)[0]
            hi = big_pre + _split(i * _BIG_16, 16)[0]
            lax.fori_loop(lo, jnp.minimum(hi, n_big), lambda k, _: start_big(k), None)
            g, r = _split(i, group_steps)
            pl.when(r == 0)(lambda: wait_reads(g, g))

            ids = iter(range(step_smalls))

            def tick():
                start_small(small_pre + i * step_smalls + next(ids))

            tick()
            matmul_step(i, tick)
            assert next(ids, None) is None

        lax.fori_loop(0, n1, read_step, None)

        for g in range(pl.cdiv(n1, group_steps), n_groups - 2):
            wait_reads(g, g)
        tail = _SLAB - _TAIL * _PIECE
        wait_reads(n_groups - 2, n_groups - 2, hi=tail)

        def write_step(i, started):
            ready = _split(i, write_steps)[0] * pieces
            target = jnp.minimum(ready, _W_FIRST + (i - n1) * _W_PER_STEP)
            start_writes(started, target)

            @pl.when(i == (n_groups - 2) * group_steps)
            def _():
                wait_reads(n_groups - 2, n_groups, lo=tail)
                wait_reads(n_groups - 1, n_groups - 1)

            matmul_step(i, lambda: None)
            return target

        started = lax.fori_loop(n1, n_steps, write_step, jnp.int32(0))
        start_writes(started, n_writes)
        pltpu.make_async_copy(buf, o_hbm, sems.at[1]).wait()

    lines = x.reshape(M // 8, 8, blocks, 128).swapaxes(1, 2)
    out = pl.pallas_call(
        kernel_function,
        in_specs=[
            pl.BlockSpec(memory_space=pl.ANY),
            pl.BlockSpec(memory_space=pl.ANY),
        ],
        out_specs=pl.BlockSpec(memory_space=pl.ANY),
        out_shape=jax.ShapeDtypeStruct((n_slabs, _SLAB, 128), x.dtype),
        scratch_shapes=[
            pltpu.VMEM((n_slabs, _SLAB, 128), x.dtype),
            pltpu.VMEM((C, C), w.dtype),
            pltpu.SemaphoreType.DMA((n_groups + 1,)),
            pltpu.SemaphoreType.DMA((2,)),
        ],
        compiler_params=pltpu.CompilerParams(
            vmem_limit_bytes=120 * 2**20,
            disable_bounds_checks=True,
            disable_semaphore_checks=True,
        ),
    )(lines.reshape(n_slabs, _SLAB, 128), w.reshape(C, C))
    return out.reshape(M // 8, blocks, 8, 128).swapaxes(1, 2).reshape(B, H, W, C)
```

```python
import jax
import jax.numpy as jnp
from jax import lax
import jax.experimental.pallas as pl
import jax.experimental.pallas.tpu as pltpu

_SLAB = 4096
_PIECE = 64
_R_SLABS = 12
_W_SLABS = 6
_SMALL = 32
_TM = 1024
_CHUNK = 128

_SPLIT = 3
_LEAD = 9
_PRE = 71
_BOOST = 11
_BIG_16 = 101
_TAIL = 2
_W_FIRST = 24
_W_PER_STEP = 14


def _split(i, n):
    assert n & (n - 1) == 0
    return lax.shift_right_logical(i, n.bit_length() - 1), i & (n - 1)


@jax.jit
def pallas_standalone__dilated_atrous__vision_kernel(
    x: jax.Array,
    w: jax.Array,
):
    B, H, W, C = x.shape
    assert w.shape == (1, 1, C, C) and C % 128 == 0
    M = B * H * W
    blocks = C // 128
    n_slabs = M * blocks // _SLAB
    n_steps = M // _TM
    chunks = _TM // _CHUNK
    pieces = _SLAB // _PIECE
    assert n_slabs * _SLAB == M * blocks and n_steps * _TM == M

    n_groups = n_slabs // _R_SLABS
    n_big = (n_groups - 1) * pieces
    n_small = _R_SLABS * _SLAB // _SMALL
    group_steps = _R_SLABS * _SLAB // (blocks * _TM)
    big_pre = _PRE + _BOOST
    small_pre = _LEAD + (_PRE - _LEAD) * _SPLIT + _BOOST
    step_smalls = chunks * (blocks - 1) + 3
    n1 = (n_small - small_pre) // step_smalls
    assert n_groups * _R_SLABS == n_slabs and group_steps * n_groups == n_steps
    assert small_pre + n1 * step_smalls == n_small
    assert big_pre + (n1 - 1) * _BIG_16 // 16 >= n_big
    assert pl.cdiv(n1, group_steps) <= n_groups - 2
    assert big_pre >= pieces and group_steps * _BIG_16 // 16 >= pieces

    n_writes = n_slabs // _W_SLABS * pieces
    write_steps = _W_SLABS * _SLAB // (blocks * _TM)
    assert write_steps * n_slabs == n_steps * _W_SLABS
    assert _W_FIRST <= n1 // write_steps * pieces

    def kernel_function(x_hbm, w_hbm, o_hbm, buf, wbuf, in_sems, sems):
        def read(idx, sem):
            return pltpu.make_async_copy(x_hbm.at[idx], buf.at[idx], in_sems.at[sem])

        def piece(j):
            return pl.ds(pl.multiple_of(j * _PIECE, _PIECE), _PIECE)

        def start_big(k):
            g, j = _split(k, pieces)
            sem = jnp.where(k >= n_big - _TAIL, n_groups, g)
            read((pl.ds(g * _R_SLABS, _R_SLABS), piece(j)), sem).start(priority=1)

        def start_part(k, part):
            g, j = _split(k, pieces)
            n = _R_SLABS // _SPLIT
            read((pl.ds(g * _R_SLABS + part * n, n), piece(j)), g).start(priority=1)

        def start_small(m):
            m, r = _split(m, _PIECE // _SMALL)
            m, s = _split(m, 2)
            pair, j = _split(m, pieces)
            lines = pl.ds(pl.multiple_of(j * _PIECE + r * _SMALL, _SMALL), _SMALL)
            read((n_slabs - _R_SLABS + 2 * pair + s, lines), n_groups - 1).start()

        def wait_reads(g, sem, lo=0, hi=_SLAB):
            read((pl.ds(g * _R_SLABS, _R_SLABS), pl.ds(lo, hi - lo)), sem).wait()

        def start_writes(lo, hi):
            def start(k, _):
                g, j = _split(k, pieces)
                idx = (pl.ds(g * _W_SLABS, _W_SLABS), piece(j))
                pltpu.make_async_copy(buf.at[idx], o_hbm.at[idx], sems.at[1]).start()

            lax.fori_loop(lo, hi, start, None)

        def matmul_step(i, tick):
            def run(k, n):
                s, r = _split((i * chunks + k) * blocks + n, _SLAB // _CHUNK)
                return s, pl.ds(pl.multiple_of(r * _CHUNK, _CHUNK), _CHUNK)

            def product(k):
                lines = jnp.concatenate([buf[run(k, n)] for n in range(blocks)])
                tiles = lines.reshape(_CHUNK // 16, 16 * blocks, 128)
                cols = [
                    jnp.concatenate(
                        [tiles[:, 8 * t:8 * t + 8] for t in (c, blocks + c)], axis=1
                    ).reshape(_CHUNK, 128)
                    for c in range(blocks)
                ]
                return jnp.dot(jnp.concatenate(cols, axis=1), wbuf[...],
                               preferred_element_type=jnp.float32)

            def store(k, res):
                tiles = [res[:, c * 128:(c + 1) * 128].reshape(_CHUNK // 8, 8, 128)
                         for c in range(blocks)]
                lines = jnp.concatenate(tiles, axis=1).reshape(blocks * _CHUNK, 128)
                lines = lines.astype(buf.dtype)
                for n in range(blocks):
                    if n < blocks - 1:
                        tick()
                    buf[run(k, n)] = lines[n * _CHUNK:(n + 1) * _CHUNK]

            res = product(0)
            tick()
            for k in range(1, chunks):
                res, done = product(k), res
                store(k - 1, done)
            store(chunks - 1, res)
            tick()

        w_copy = pltpu.make_async_copy(w_hbm, wbuf, sems.at[0])
        w_copy.start(priority=1)

        def lead(k, _):
            for part in range(_SPLIT):
                start_part(k, part)
            start_small(k)

        def pre(k, _):
            for part in range(_SPLIT):
                start_part(k, part)
                start_small(_LEAD + (k - _LEAD) * _SPLIT + part)

        def boost(k, _):
            start_big(_PRE + k)
            start_small(small_pre - _BOOST + k)

        lax.fori_loop(0, _LEAD, lead, None)
        lax.fori_loop(_LEAD, _PRE, pre, None)
        lax.fori_loop(0, _BOOST, boost, None)
        w_copy.wait()

        def read_step(i, _):
            lo = big_pre + _split(jnp.maximum(i - 1, 0) * _BIG_16, 16)[0]
            hi = big_pre + _split(i * _BIG_16, 16)[0]
            lax.fori_loop(lo, jnp.minimum(hi, n_big), lambda k, _: start_big(k), None)
            g, r = _split(i, group_steps)
            pl.when(r == 0)(lambda: wait_reads(g, g))

            ids = iter(range(step_smalls))

            def tick():
                start_small(small_pre + i * step_smalls + next(ids))

            tick()
            matmul_step(i, tick)
            assert next(ids, None) is None

        lax.fori_loop(0, n1, read_step, None)

        for g in range(pl.cdiv(n1, group_steps), n_groups - 2):
            wait_reads(g, g)
        tail = _SLAB - _TAIL * _PIECE
        wait_reads(n_groups - 2, n_groups - 2, hi=tail)

        def write_step(i, started):
            ready = _split(i, write_steps)[0] * pieces
            target = jnp.minimum(ready, _W_FIRST + (i - n1) * _W_PER_STEP)
            start_writes(started, target)

            @pl.when(i == (n_groups - 2) * group_steps)
            def _():
                wait_reads(n_groups - 2, n_groups, lo=tail)
                wait_reads(n_groups - 1, n_groups - 1)

            matmul_step(i, lambda: None)
            return target

        started = lax.fori_loop(n1, n_steps, write_step, jnp.int32(0))
        start_writes(started, n_writes)
        pltpu.make_async_copy(buf, o_hbm, sems.at[1]).wait()

    lines = x.reshape(M // 8, 8, blocks, 128).swapaxes(1, 2)
    out = pl.pallas_call(
        kernel_function,
        in_specs=[
            pl.BlockSpec(memory_space=pl.ANY),
            pl.BlockSpec(memory_space=pl.ANY),
        ],
        out_specs=pl.BlockSpec(memory_space=pl.ANY),
        out_shape=jax.ShapeDtypeStruct((n_slabs, _SLAB, 128), x.dtype),
        scratch_shapes=[
            pltpu.VMEM((n_slabs, _SLAB, 128), x.dtype),
            pltpu.VMEM((C, C), w.dtype),
            pltpu.SemaphoreType.DMA((n_groups + 1,)),
            pltpu.SemaphoreType.DMA((2,)),
        ],
        compiler_params=pltpu.CompilerParams(
            vmem_limit_bytes=120 * 2**20,
            disable_bounds_checks=True,
            disable_semaphore_checks=True,
        ),
    )(lines.reshape(n_slabs, _SLAB, 128), w.reshape(C, C))
    return out.reshape(M // 8, blocks, 8, 128).swapaxes(1, 2).reshape(B, H, W, C)
```
